```python
import os as _os
_os.environ.setdefault("JAX_PLATFORMS", "cpu")
import jax
import jax.numpy as jnp

def _softmax(x, axis=-1):
    return jax.nn.softmax(x, axis=axis)
def _gelu(x):
    return jax.nn.gelu(x, approximate=True)
def _silu(x):
    return jax.nn.silu(x)
def _sigmoid(x):
    return jax.nn.sigmoid(x)
def _layernorm(x, axis=-1, eps=1e-5):
    m = jnp.mean(x, axis=axis, keepdims=True)
    v = jnp.var(x, axis=axis, keepdims=True)
    return (x - m) / jnp.sqrt(v + eps)
def _scatter_add(tgt, idx, src, axis=0):
    return tgt.at[idx].add(src)
def _segment_sum(src, seg, n):
    return jax.ops.segment_sum(src, seg, n)
class _Rng:
    def __init__(self, key):
        self._k = key
    def _next(self):
        self._k, sub = jax.random.split(self._k)
        return sub
    def normal(self, shape):
        return jax.random.normal(self._next(), shape, dtype=jnp.bfloat16)
    def randint(self, lo, hi, shape):
        return jax.random.randint(self._next(), shape, lo, hi, dtype=jnp.int32)
    def uniform(self, shape, lo=0.0, hi=1.0):
        return jax.random.uniform(self._next(), shape, jnp.bfloat16, lo, hi)
    def permutation(self, n):
        return jax.random.permutation(self._next(), n)


kernel_name = 'interleave_layers__sliding_block__dense_activation_gelu__prompt'

def setup_inputs():
    _rng = _Rng(jax.random.key(int.from_bytes(__import__("os").urandom(4), "little")))
    _w = (lambda a: (lambda t: t.astype(jnp.bfloat16) if jnp.issubdtype(t.dtype, jnp.floating) else t)(jnp.asarray(a)))
    def _A_setup():
        B, S, D = 1, 2048, 640
        return {
            "x": _w((lambda *s: _rng.normal(s) * 0.05)(B, S, D)),
            "wqkv": _w((lambda *s: _rng.normal(s) * 0.05)(D, 3 * D)),
            "wo": _w((lambda *s: _rng.normal(s) * 0.05)(D, D)),
        }
    _A_in = _A_setup()

    def _B_setup():
        B, S, D, F = 1, 2048, 640, 1728
        return {
            "x": _w((lambda *s: _rng.normal(s) * 0.05)(B, S, D)),
            "w1": _w((lambda *s: _rng.normal(s) * 0.8)(D, F) * (D ** -0.5)),
            "b1": _w((lambda *s: _rng.normal(s) * 0.8)(F) * 0.01),
            "w2": _w((lambda *s: _rng.normal(s) * 0.8)(F, D) * (F ** -0.5)),
            "b2": _w((lambda *s: _rng.normal(s) * 0.8)(D) * 0.01),
        }
    _B_in = _B_setup()

    return {
        "A_x": _A_in["x"],
        "A_wqkv": _A_in["wqkv"],
        "A_wo": _A_in["wo"],
        "B_x": _B_in["x"],
        "B_w1": _B_in["w1"],
        "B_b1": _B_in["b1"],
        "B_w2": _B_in["w2"],
        "B_b2": _B_in["b2"],
    }

def reference(A_x, A_wqkv, A_wo, B_x, B_w1, B_b1, B_w2, B_b2):
    def _A_ref(x, wqkv, wo):
        B, S, D = x.shape
        H = 32; Dh = D // H; W = 256
        qkv = (lambda x, *d: x.transpose(*d))((x @ wqkv).reshape(B, S, 3, H, Dh), 2, 0, 3, 1, 4)
        q, k, v = qkv[0], qkv[1], qkv[2]
        scores = jnp.einsum("bhqd,bhkd->bhqk", q, k) * (Dh ** -0.5)
        idx = jnp.arange(S)
        mask = (idx[:, None] - idx[None, :] >= 0) & (idx[:, None] - idx[None, :] < W)
        scores = jnp.where(mask[None, None], scores, -1e9)
        p = _softmax(scores, axis=-1)
        o = jnp.einsum("bhqk,bhkd->bhqd", p, v)
        return (lambda x, *d: x.transpose(*d))(o, 0, 2, 1, 3).reshape(B, S, D) @ wo

    def _B_ref(x, w1, b1, w2, b2):
        h = jnp.einsum("bsd,df->bsf", x, w1) + b1
        h = _gelu(h)
        return jnp.einsum("bsf,fd->bsd", h, w2) + b2

    x = A_x
    x = x + _A_ref(_layernorm(x, axis=-1), A_wqkv, A_wo)
    x = x + _B_ref(_layernorm(x, axis=-1), B_w1, B_b1, B_w2, B_b2)
    x = x + _A_ref(_layernorm(x, axis=-1), A_wqkv, A_wo)
    x = x + _B_ref(_layernorm(x, axis=-1), B_w1, B_b1, B_w2, B_b2)
    return x
```

```python
import numpy as np
import jax
import jax.numpy as jnp
from jax import lax
import jax.experimental.pallas as pl
import jax.experimental.pallas.tpu as pltpu

S, D, H, DH, W, F = 2048, 640, 32, 20, 256, 1728
BQ = 128
HP = 24
RB = 512
NG = D // 128
NT = (((1,), (1,)), ((), ()))
TN = (((0,), (0,)), ((), ()))
f32, bf16 = jnp.float32, jnp.bfloat16


def _ln(x):
    m = jnp.mean(x, axis=-1, keepdims=True)
    xc = x - m
    v = jnp.mean(xc * xc, axis=-1, keepdims=True)
    return xc * lax.rsqrt(v + 1e-5)


def _gelu(x):
    c = np.float32(np.sqrt(2.0 / np.pi))
    return 0.5 * x * (1.0 + jnp.tanh(c * (x + 0.044715 * (x * x * x))))


def _kernel(x_ref, wqkv_ref, wo_hbm, w1t_hbm, b1_ref, w2_hbm, b2_ref, o_ref,
            xs, q_s, k_s, vt_s, ot_s, wvt_s, cap_s, wo_s, w1t_s, w2_s, sems):
    cps = [pltpu.make_async_copy(wo_hbm, wo_s, sems.at[0]),
           pltpu.make_async_copy(w1t_hbm, w1t_s, sems.at[1]),
           pltpu.make_async_copy(w2_hbm, w2_s, sems.at[2])]
    for cp in cps:
        cp.start()

    wvt = jnp.transpose(wqkv_ref[:, 2 * D:3 * D].astype(f32))
    for h in range(H):
        wvt_s[HP * h:HP * h + HP, :] = jnp.concatenate(
            [wvt[DH * h:DH * h + DH, :], jnp.zeros((HP - DH, D), f32)], axis=0)
    k_s[:, 0:W, :] = jnp.zeros((NG, W, 128), bf16)
    vt_s[:, :, 0:W] = jnp.zeros((H, 32, W), bf16)

    def p1(i, xsrc):
        r0 = pl.multiple_of(i * RB, RB)
        xn = _ln(xsrc[pl.ds(r0, RB), :].astype(f32)).astype(bf16)
        qk = jnp.dot(xn, wqkv_ref[:, 0:2 * D], preferred_element_type=f32)
        for g in range(NG):
            q_s[g, pl.ds(r0, RB), :] = (qk[:, 128 * g:128 * g + 128]
                                        * np.float32(DH ** -0.5 * np.log2(np.e))).astype(bf16)
            k_s[g, pl.ds(W + r0, RB), :] = qk[:, D + 128 * g:D + 128 * g + 128].astype(bf16)
        vt = lax.dot_general(wvt_s[...].astype(bf16), xn, NT, preferred_element_type=f32)
        row = lax.broadcasted_iota(jnp.int32, (HP, RB), 0)
        zpad = jnp.zeros((32 - HP, RB), f32)
        for h in range(H):
            blk = jnp.where(row == DH, 1.0, vt[HP * h:HP * h + HP, :])
            vt_s[h, :, pl.ds(W + r0, RB)] = jnp.concatenate([blk, zpad], axis=0).astype(bf16)

    def p2(i, mask_mid):
        q0 = pl.multiple_of(i * BQ, BQ)
        kr = lax.broadcasted_iota(jnp.int32, (W + BQ, BQ), 0)
        qc = lax.broadcasted_iota(jnp.int32, (W + BQ, BQ), 1)
        dlt = qc + W - kr
        valid = (dlt >= 0) & (dlt < W) & (kr + q0 >= W)
        cap_s[...] = jnp.where(valid, 3e38, -1e9).astype(f32)
        lane = lax.broadcasted_iota(jnp.int32, (BQ // 2, 128), 1)
        partial = {}
        for g in range(NG):
            hs = [h for h in range(H) if DH * h < 128 * (g + 1) and DH * h + DH > 128 * g]
            qg = pltpu.bitcast(q_s[g, pl.ds(q0, BQ), :], jnp.uint32)
            kg = k_s[g, pl.ds(q0, W + BQ), :]
            qms = []
            for h in hs:
                lo, hi = DH * h - 128 * g, DH * h + DH - 128 * g
                qms.append(jnp.where((lane >= lo) & (lane < hi), qg, jnp.zeros_like(qg)))
            qm = pltpu.bitcast(jnp.concatenate(qms, axis=0), bf16)
            sall = lax.dot_general(kg, qm, NT, preferred_element_type=f32)
            for j, h in enumerate(hs):
                st = sall[:, 128 * j:128 * j + 128]
                if h in partial:
                    st = st + partial.pop(h)
                elif DH * h + DH > 128 * (g + 1):
                    partial[h] = st
                    continue
                sa = jnp.minimum(st[0:BQ], cap_s[0:BQ, :])
                sb = jnp.minimum(st[BQ:W], cap_s[BQ:W, :]) if mask_mid else st[BQ:W]
                sc = jnp.minimum(st[W:], cap_s[W:, :])
                m = jnp.max(jnp.maximum(jnp.maximum(sa, sb), sc), axis=0, keepdims=True)
                p = jnp.concatenate([jnp.exp2(sa - m), jnp.exp2(sb - m), jnp.exp2(sc - m)], axis=0).astype(bf16)
                ov = jnp.dot(vt_s[h, :, pl.ds(q0, W + BQ)], p, preferred_element_type=f32)
                ot_s[DH * h:DH * h + DH, pl.ds(q0, BQ)] = ov[0:DH, :] * (1.0 / ov[DH:DH + 1, :])

    def p3(i, xsrc, dst):
        r0 = pl.multiple_of(i * RB, RB)
        ot = ot_s[:, pl.ds(r0, RB)].astype(bf16)
        a = lax.dot_general(ot, wo_s[...], TN, preferred_element_type=f32)
        x1 = xsrc[pl.ds(r0, RB), :].astype(f32) + a
        xn = _ln(x1).astype(bf16)
        hh = lax.dot_general(xn, w1t_s[...], NT, preferred_element_type=f32) + b1_ref[...].astype(f32)
        hh = _gelu(hh).astype(bf16)
        y = jnp.dot(hh, w2_s[...], preferred_element_type=f32) + b2_ref[...].astype(f32)
        dst[pl.ds(r0, RB), :] = (x1 + y).astype(dst.dtype)

    def loop(n0, n1, fn):
        def body(i, c):
            fn(i)
            return c
        lax.fori_loop(n0, n1, body, 0)

    for layer in range(2):
        xsrc = x_ref if layer == 0 else xs
        dst = xs if layer == 0 else o_ref
        loop(0, S // RB, lambda i: p1(i, xsrc))
        p2(0, True)
        loop(1, S // BQ, lambda i: p2(i, False))
        if layer == 0:
            for cp in cps:
                cp.wait()
        loop(0, S // RB, lambda i: p3(i, xsrc, dst))


@jax.jit
def pallas_interleave_layers__sliding_block__dense_activation_gelu__prompt_kernel(A_x, A_wqkv, A_wo, B_x, B_w1, B_b1, B_w2, B_b2):
    del B_x
    vm = pl.BlockSpec(memory_space=pltpu.VMEM)
    hbm = pl.BlockSpec(memory_space=pl.ANY)
    out = pl.pallas_call(
        _kernel,
        out_shape=jax.ShapeDtypeStruct((S, D), bf16),
        in_specs=[vm, vm, hbm, hbm, vm, hbm, vm],
        out_specs=vm,
        scratch_shapes=[
            pltpu.VMEM((S, D), f32),
            pltpu.VMEM((NG, S, 128), bf16),
            pltpu.VMEM((NG, W + S, 128), bf16),
            pltpu.VMEM((H, 32, W + S), bf16),
            pltpu.VMEM((D, S), f32),
            pltpu.VMEM((H * HP, D), f32),
            pltpu.VMEM((W + BQ, BQ), f32),
            pltpu.VMEM((D, D), bf16),
            pltpu.VMEM((F, D), bf16),
            pltpu.VMEM((F, D), bf16),
            pltpu.SemaphoreType.DMA((3,)),
        ],
        compiler_params=pltpu.CompilerParams(vmem_limit_bytes=100 * 1024 * 1024),
    )(A_x.reshape(S, D), A_wqkv, A_wo, B_w1.T, B_b1.reshape(1, F), B_w2, B_b2.reshape(1, D))
    return out.reshape(1, S, D)
```

```python
import numpy as np
import jax
import jax.numpy as jnp
from jax import lax
import jax.experimental.pallas as pl
import jax.experimental.pallas.tpu as pltpu

S, D, H, DH, W, F = 2048, 640, 32, 20, 256, 1728
BQ = 128
import os
LA = int('8')
NR = LA + 1
HP = 24
RB = 512
NG = D // 128
STR = [h for h in range(H) if (DH * h) // 128 != (DH * h + DH - 1) // 128]
NT = (((1,), (1,)), ((), ()))
TN = (((0,), (0,)), ((), ()))
f32, bf16 = jnp.float32, jnp.bfloat16


def _ln(x):
    m = jnp.mean(x, axis=-1, keepdims=True)
    xc = x - m
    v = jnp.mean(xc * xc, axis=-1, keepdims=True)
    return xc * lax.rsqrt(v + 1e-5)


def _gelu(x):
    c = np.float32(np.sqrt(2.0 / np.pi))
    return 0.5 * x * (1.0 + jnp.tanh(c * (x + 0.044715 * (x * x * x))))


def _kernel(x_hbm, wqkv_hbm, wo_hbm, w1t_hbm, b1_ref, w2_hbm, b2_ref, o_hbm,
            xs, q_s, k_s, vt_s, ot_s, wvt_s, cap_s, wo_s, w1t_s, w2_s, s_buf, x_ref, wqk_s, wv_s, o_ref, sems):
    NB = S // RB

    def x_cp(i):
        r = pl.ds(pl.multiple_of(i * RB, RB), RB)
        return pltpu.make_async_copy(x_hbm.at[r, :], x_ref.at[r, :], sems.at[i])

    def o_cp(i):
        r = pl.ds(pl.multiple_of(i * RB, RB), RB)
        return pltpu.make_async_copy(o_ref.at[r, :], o_hbm.at[r, :], sems.at[NB + i])

    wv_cp = pltpu.make_async_copy(wqkv_hbm.at[:, 2 * D:3 * D], wv_s, sems.at[2 * NB])
    wqk_cp = pltpu.make_async_copy(wqkv_hbm.at[:, 0:2 * D], wqk_s, sems.at[2 * NB + 1])
    cps = [pltpu.make_async_copy(wo_hbm, wo_s, sems.at[2 * NB + 2]),
           pltpu.make_async_copy(w1t_hbm, w1t_s, sems.at[2 * NB + 3]),
           pltpu.make_async_copy(w2_hbm, w2_s, sems.at[2 * NB + 4])]
    wv_cp.start()
    x_cp(0).start()
    wqk_cp.start()
    for i in range(1, NB):
        x_cp(i).start()
    for cp in cps:
        cp.start()
    k_s[:, 0:W, :] = jnp.zeros((NG + 1, W, 128), bf16)
    vt_s[:, :, 0:W] = jnp.zeros((H, 32, W), bf16)
    wv_cp.wait()
    wvt = jnp.transpose(wv_s[...].astype(f32))
    wvt_s[...] = wvt.astype(bf16)
    wqk_cp.wait()

    def p1(i, xsrc):
        r0 = pl.multiple_of(i * RB, RB)
        xn = _ln(xsrc[pl.ds(r0, RB), :].astype(f32)).astype(bf16)
        qk = jnp.dot(xn, wqk_s[...], preferred_element_type=f32)
        for g in range(NG):
            q_s[g, pl.ds(r0, RB), :] = (qk[:, 128 * g:128 * g + 128]
                                        * np.float32(DH ** -0.5 * np.log2(np.e))).astype(bf16)
            k_s[g, pl.ds(W + r0, RB), :] = qk[:, D + 128 * g:D + 128 * g + 128].astype(bf16)
        zl = jnp.zeros((RB, 128 - DH * len(STR)), f32)
        q_s[NG, pl.ds(r0, RB), :] = (jnp.concatenate([qk[:, DH * h:DH * h + DH] for h in STR] + [zl], axis=1)
                                     * np.float32(DH ** -0.5 * np.log2(np.e))).astype(bf16)
        k_s[NG, pl.ds(W + r0, RB), :] = jnp.concatenate(
            [qk[:, D + DH * h:D + DH * h + DH] for h in STR] + [zl], axis=1).astype(bf16)
        vt = lax.dot_general(wvt_s[...], xn, NT, preferred_element_type=f32)
        row = lax.broadcasted_iota(jnp.int32, (32 - DH, RB), 0)
        tail = jnp.where(row == 0, 1.0, 0.0).astype(f32)
        for h in range(H):
            vt_s[h, :, pl.ds(W + r0, RB)] = jnp.concatenate([vt[DH * h:DH * h + DH, :], tail], axis=0).astype(bf16)

    def p2(i, mask_mid):
        q0 = pl.multiple_of(i * BQ, BQ)
        kr = lax.broadcasted_iota(jnp.int32, (W + BQ, BQ), 0)
        qc = lax.broadcasted_iota(jnp.int32, (W + BQ, BQ), 1)
        dlt = qc + W - kr
        valid = (dlt >= 0) & (dlt < W) & (kr + q0 >= W)
        cap_s[...] = jnp.where(valid, 3e38, -1e9).astype(f32)
        lane = lax.broadcasted_iota(jnp.int32, (BQ // 2, 128), 1)

        def qk(h):
            if h in STR:
                g, lo = NG, DH * STR.index(h)
            else:
                g, lo = (DH * h) // 128, (DH * h) % 128
            qg = pltpu.bitcast(q_s[g, pl.ds(q0, BQ), :], jnp.uint32)
            qm = jnp.where((lane >= lo) & (lane < lo + DH), qg, jnp.zeros_like(qg))
            s_buf[h % NR] = lax.dot_general(k_s[g, pl.ds(q0, W + BQ), :], pltpu.bitcast(qm, bf16), NT,
                                            preferred_element_type=f32)

        def sm(h):
            st = s_buf.at[h % NR]
            sa = jnp.minimum(st[0:BQ, :], cap_s[0:BQ, :])
            sb = jnp.minimum(st[BQ:W, :], cap_s[BQ:W, :]) if mask_mid else st[BQ:W, :]
            sc = jnp.minimum(st[W:, :], cap_s[W:, :])
            m = jnp.max(jnp.maximum(jnp.maximum(sa, sb), sc), axis=0, keepdims=True)
            p = jnp.concatenate([jnp.exp2(sa - m), jnp.exp2(sb - m), jnp.exp2(sc - m)], axis=0).astype(bf16)
            ov = jnp.dot(vt_s[h, :, pl.ds(q0, W + BQ)], p, preferred_element_type=f32)
            ot_s[DH * h:DH * h + DH, pl.ds(q0, BQ)] = ov[0:DH, :] * (1.0 / ov[DH:DH + 1, :])

        for h in range(LA):
            qk(h)
        for h in range(H):
            if h + LA < H:
                qk(h + LA)
            sm(h)

    def p3(i, xsrc, dst):
        r0 = pl.multiple_of(i * RB, RB)
        ot = ot_s[:, pl.ds(r0, RB)].astype(bf16)
        a = lax.dot_general(ot, wo_s[...], TN, preferred_element_type=f32)
        x1 = xsrc[pl.ds(r0, RB), :].astype(f32) + a
        xn = _ln(x1).astype(bf16)
        hh = lax.dot_general(xn, w1t_s[...], NT, preferred_element_type=f32) + b1_ref[...].astype(f32).reshape(1, F)
        hh = _gelu(hh).astype(bf16)
        y = jnp.dot(hh, w2_s[...], preferred_element_type=f32) + b2_ref[...].astype(f32).reshape(1, D)
        dst[pl.ds(r0, RB), :] = (x1 + y).astype(dst.dtype)

    def loop(n0, n1, fn):
        def body(i, c):
            fn(i)
            return c
        lax.fori_loop(n0, n1, body, 0)

    for layer in range(2):
        xsrc = x_ref if layer == 0 else xs
        dst = xs if layer == 0 else o_ref
        def p1w(i):
            if layer == 0:
                x_cp(i).wait()
            p1(i, xsrc)
        loop(0, NB, p1w)
        p2(0, True)
        loop(1, S // BQ, lambda i: p2(i, False))
        if layer == 0:
            for cp in cps:
                cp.wait()
        def p3w(i):
            p3(i, xsrc, dst)
            if layer == 1:
                o_cp(i).start()
        loop(0, NB, p3w)
    for i in range(NB):
        o_cp(i).wait()


@jax.jit
def pallas_interleave_layers__sliding_block__dense_activation_gelu__prompt_kernel(A_x, A_wqkv, A_wo, B_x, B_w1, B_b1, B_w2, B_b2):
    del B_x
    vm = pl.BlockSpec(memory_space=pltpu.VMEM)
    hbm = pl.BlockSpec(memory_space=pl.ANY)
    out = pl.pallas_call(
        _kernel,
        out_shape=jax.ShapeDtypeStruct((S, D), bf16),
        in_specs=[hbm, hbm, hbm, hbm, vm, hbm, vm],
        out_specs=hbm,
        scratch_shapes=[
            pltpu.VMEM((S, D), f32),
            pltpu.VMEM((NG + 1, S, 128), bf16),
            pltpu.VMEM((NG + 1, W + S, 128), bf16),
            pltpu.VMEM((H, 32, W + S), bf16),
            pltpu.VMEM((D, S), f32),
            pltpu.VMEM((D, D), bf16),
            pltpu.VMEM((W + BQ, BQ), f32),
            pltpu.VMEM((D, D), bf16),
            pltpu.VMEM((F, D), bf16),
            pltpu.VMEM((F, D), bf16),
            pltpu.VMEM((NR, W + BQ, BQ), f32),
            pltpu.VMEM((S, D), bf16),
            pltpu.VMEM((D, 2 * D), bf16),
            pltpu.VMEM((D, D), bf16),
            pltpu.VMEM((S, D), bf16),
            pltpu.SemaphoreType.DMA((2 * (S // RB) + 5,)),
        ],
        compiler_params=pltpu.CompilerParams(vmem_limit_bytes=100 * 1024 * 1024),
    )(A_x.reshape(S, D), A_wqkv, A_wo, B_w1.T, B_b1, B_w2, B_b2)
    return out.reshape(1, S, D)
```

```python
import functools
import numpy as np
import jax
import jax.numpy as jnp
from jax import lax
import jax.experimental.pallas as pl
import jax.experimental.pallas.tpu as pltpu

S, D, H, DH, W, F = 2048, 640, 32, 20, 256, 1728
BQ = 128

LA = 8
NR = LA + 1
HP = 24
RB = 512
NG = D // 128
STR = [h for h in range(H) if (DH * h) // 128 != (DH * h + DH - 1) // 128]
NT = (((1,), (1,)), ((), ()))
TN = (((0,), (0,)), ((), ()))
f32, bf16 = jnp.float32, jnp.bfloat16


def _ln(x):
    m = jnp.mean(x, axis=-1, keepdims=True)
    xc = x - m
    v = jnp.mean(xc * xc, axis=-1, keepdims=True)
    return xc * lax.rsqrt(v + 1e-5)


def _gelu(x):
    c = np.float32(np.sqrt(2.0 / np.pi))
    return 0.5 * x * (1.0 + jnp.tanh(c * (x + 0.044715 * (x * x * x))))


def _kernel(x_hbm, wqkv_hbm, wo_hbm, w1t_hbm, b1_ref, w2_hbm, b2_ref, o_hbm,
            xs, q_s, k_s, vt_s, ot_s, wvt_s, cap_s, wo_s, w1t_s, w2_s, s_buf, x_ref, wqk_s, wv_s, o_ref, x1_s, xn_s, h_s, sems):
    NB = S // RB

    def x_cp(i):
        r = pl.ds(pl.multiple_of(i * RB, RB), RB)
        return pltpu.make_async_copy(x_hbm.at[r, :], x_ref.at[r, :], sems.at[i])

    def o_cp(i):
        r = pl.ds(pl.multiple_of(i * 256, 256), 256)
        return pltpu.make_async_copy(o_ref.at[r, :], o_hbm.at[r, :], sems.at[NB + 5 + i])

    wv_cp = pltpu.make_async_copy(wqkv_hbm.at[:, 2 * D:3 * D], wv_s, sems.at[NB])
    wqk_cp = pltpu.make_async_copy(wqkv_hbm.at[:, 0:2 * D], wqk_s, sems.at[NB + 1])
    cps = [pltpu.make_async_copy(wo_hbm, wo_s, sems.at[NB + 2]),
           pltpu.make_async_copy(w1t_hbm, w1t_s, sems.at[NB + 3]),
           pltpu.make_async_copy(w2_hbm, w2_s, sems.at[NB + 4])]
    wv_cp.start()
    x_cp(0).start()
    wqk_cp.start()
    for i in range(1, NB):
        x_cp(i).start()
    for cp in cps:
        cp.start()
    k_s[:, 0:W, :] = jnp.zeros((NG + 1, W, 128), bf16)
    vt_s[:, :, 0:W] = jnp.zeros((H, 32, W), bf16)
    wv_cp.wait()
    wvt = jnp.transpose(wv_s[...].astype(f32))
    wvt_s[...] = wvt.astype(bf16)
    wqk_cp.wait()

    def p1(i, xsrc):
        r0 = pl.multiple_of(i * RB, RB)
        xn = _ln(xsrc[pl.ds(r0, RB), :].astype(f32)).astype(bf16)
        qk = jnp.dot(xn, wqk_s[...], preferred_element_type=f32)
        for g in range(NG):
            q_s[g, pl.ds(r0, RB), :] = (qk[:, 128 * g:128 * g + 128]
                                        * np.float32(DH ** -0.5 * np.log2(np.e))).astype(bf16)
            k_s[g, pl.ds(W + r0, RB), :] = qk[:, D + 128 * g:D + 128 * g + 128].astype(bf16)
        zl = jnp.zeros((RB, 128 - DH * len(STR)), f32)
        q_s[NG, pl.ds(r0, RB), :] = (jnp.concatenate([qk[:, DH * h:DH * h + DH] for h in STR] + [zl], axis=1)
                                     * np.float32(DH ** -0.5 * np.log2(np.e))).astype(bf16)
        k_s[NG, pl.ds(W + r0, RB), :] = jnp.concatenate(
            [qk[:, D + DH * h:D + DH * h + DH] for h in STR] + [zl], axis=1).astype(bf16)
        vt = lax.dot_general(wvt_s[...], xn, NT, preferred_element_type=f32)
        row = lax.broadcasted_iota(jnp.int32, (32 - DH, RB), 0)
        tail = jnp.where(row == 0, 1.0, 0.0).astype(f32)
        for h in range(H):
            vt_s[h, :, pl.ds(W + r0, RB)] = jnp.concatenate([vt[DH * h:DH * h + DH, :], tail], axis=0).astype(bf16)

    def p2(i, mask_mid, hook=None):
        q0 = pl.multiple_of(i * BQ, BQ)
        kr = lax.broadcasted_iota(jnp.int32, (W + BQ, BQ), 0)
        qc = lax.broadcasted_iota(jnp.int32, (W + BQ, BQ), 1)
        dlt = qc + W - kr
        valid = (dlt >= 0) & (dlt < W) & (kr + q0 >= W)
        cap_s[...] = jnp.where(valid, 3e38, -1e9).astype(f32)
        lane = lax.broadcasted_iota(jnp.int32, (BQ // 2, 128), 1)

        def qk(h):
            if h in STR:
                g, lo = NG, DH * STR.index(h)
            else:
                g, lo = (DH * h) // 128, (DH * h) % 128
            qg = pltpu.bitcast(q_s[g, pl.ds(q0, BQ), :], jnp.uint32)
            qm = jnp.where((lane >= lo) & (lane < lo + DH), qg, jnp.zeros_like(qg))
            s_buf[h % NR] = lax.dot_general(k_s[g, pl.ds(q0, W + BQ), :], pltpu.bitcast(qm, bf16), NT,
                                            preferred_element_type=f32)

        def sm(h):
            st = s_buf.at[h % NR]
            sa = jnp.minimum(st[0:BQ, :], cap_s[0:BQ, :])
            sb = jnp.minimum(st[BQ:W, :], cap_s[BQ:W, :]) if mask_mid else st[BQ:W, :]
            sc = jnp.minimum(st[W:, :], cap_s[W:, :])
            m = jnp.max(jnp.maximum(jnp.maximum(sa, sb), sc), axis=0, keepdims=True)
            p = jnp.concatenate([jnp.exp2(sa - m), jnp.exp2(sb - m), jnp.exp2(sc - m)], axis=0).astype(bf16)
            ov = jnp.dot(vt_s[h, :, pl.ds(q0, W + BQ)], p, preferred_element_type=f32)
            ot_s[DH * h:DH * h + DH, pl.ds(q0, BQ)] = ov[0:DH, :] * (1.0 / ov[DH:DH + 1, :])

        for h in range(LA):
            qk(h)
        for h in range(H):
            if h + LA < H:
                qk(h + LA)
            sm(h)
            if hook is not None:
                hook(h)

    def p3(i, xsrc, dst):
        r0 = pl.multiple_of(i * RB, RB)
        ot = ot_s[:, pl.ds(r0, RB)].astype(bf16)
        a = lax.dot_general(ot, wo_s[...], TN, preferred_element_type=f32)
        x1 = xsrc[pl.ds(r0, RB), :].astype(f32) + a
        xn = _ln(x1).astype(bf16)
        hh = lax.dot_general(xn, w1t_s[...], NT, preferred_element_type=f32) + b1_ref[...].astype(f32).reshape(1, F)
        hh = _gelu(hh).astype(bf16)
        y = jnp.dot(hh, w2_s[...], preferred_element_type=f32) + b2_ref[...].astype(f32).reshape(1, D)
        dst[pl.ds(r0, RB), :] = (x1 + y).astype(dst.dtype)

    PB = 256

    def p3_pieces(j, xsrc, dst):
        r0 = pl.multiple_of(j * PB, PB)
        rows = pl.ds(r0, PB)
        pieces = []

        def pa():
            ot = ot_s[:, rows].astype(bf16)
            a = lax.dot_general(ot, wo_s[...], TN, preferred_element_type=f32)
            x1_s[...] = xsrc[rows, :].astype(f32) + a

        def pln():
            xn_s[...] = _ln(x1_s[...]).astype(bf16)

        def ph(c):
            lo, hi = 128 * c, min(128 * c + 128, F)
            hh = lax.dot_general(xn_s[...], w1t_s[lo:hi, :], NT, preferred_element_type=f32)
            hh = hh + b1_ref[...].astype(f32).reshape(1, F)[:, lo:hi]
            h_s[:, lo:hi] = _gelu(hh).astype(bf16)

        def py(n):
            y = jnp.dot(h_s[...], w2_s[:, 128 * n:128 * n + 128], preferred_element_type=f32)
            y = y + b2_ref[...].astype(f32).reshape(1, D)[:, 128 * n:128 * n + 128]
            dst[rows, 128 * n:128 * n + 128] = (x1_s[:, 128 * n:128 * n + 128] + y).astype(dst.dtype)

        pieces.append(pa)
        pieces.append(pln)
        for c in range((F + 127) // 128):
            pieces.append(functools.partial(ph, c))
        for n in range(NG):
            pieces.append(functools.partial(py, n))
        return pieces

    def loop(n0, n1, fn):
        def body(i, c):
            fn(i)
            return c
        lax.fori_loop(n0, n1, body, 0)

    for layer in range(2):
        xsrc = x_ref if layer == 0 else xs
        dst = xs if layer == 0 else o_ref
        def p1w(i):
            if layer == 0:
                x_cp(i).wait()
            p1(i, xsrc)
        loop(0, NB, p1w)
        p2(0, True)
        p2(1, False)
        if layer == 0:
            for cp in cps:
                cp.wait()
        SCHED = [0, 8] + list(range(12, 40, 2)) + [40, 45, 50, 55, 60]

        def fused(j):
            pcs = p3_pieces(j - 1, xsrc, dst)
            at = dict(zip(SCHED, pcs))
            for t in range(2):
                p2(2 * j + t, False, lambda h, t=t: at[32 * t + h]() if 32 * t + h in at else None)
            if layer == 1:
                o_cp(j - 1).start()
        loop(1, S // PB, fused)
        for pc in p3_pieces(S // PB - 1, xsrc, dst):
            pc()
        if layer == 1:
            o_cp(S // PB - 1).start()
    for i in range(S // PB):
        o_cp(i).wait()


@jax.jit
def pallas_interleave_layers__sliding_block__dense_activation_gelu__prompt_kernel(A_x, A_wqkv, A_wo, B_x, B_w1, B_b1, B_w2, B_b2):
    del B_x
    vm = pl.BlockSpec(memory_space=pltpu.VMEM)
    hbm = pl.BlockSpec(memory_space=pl.ANY)
    out = pl.pallas_call(
        _kernel,
        out_shape=jax.ShapeDtypeStruct((S, D), bf16),
        in_specs=[hbm, hbm, hbm, hbm, vm, hbm, vm],
        out_specs=hbm,
        scratch_shapes=[
            pltpu.VMEM((S, D), f32),
            pltpu.VMEM((NG + 1, S, 128), bf16),
            pltpu.VMEM((NG + 1, W + S, 128), bf16),
            pltpu.VMEM((H, 32, W + S), bf16),
            pltpu.VMEM((D, S), f32),
            pltpu.VMEM((D, D), bf16),
            pltpu.VMEM((W + BQ, BQ), f32),
            pltpu.VMEM((D, D), bf16),
            pltpu.VMEM((F, D), bf16),
            pltpu.VMEM((F, D), bf16),
            pltpu.VMEM((NR, W + BQ, BQ), f32),
            pltpu.VMEM((S, D), bf16),
            pltpu.VMEM((D, 2 * D), bf16),
            pltpu.VMEM((D, D), bf16),
            pltpu.VMEM((S, D), bf16),
            pltpu.VMEM((256, D), f32),
            pltpu.VMEM((256, D), bf16),
            pltpu.VMEM((256, F), bf16),
            pltpu.SemaphoreType.DMA((S // RB + 5 + S // 256,)),
        ],
        compiler_params=pltpu.CompilerParams(vmem_limit_bytes=100 * 1024 * 1024),
    )(A_x.reshape(S, D), A_wqkv, A_wo, B_w1.T, B_b1, B_w2, B_b2)
    return out.reshape(1, S, D)
```

```python
import functools
import numpy as np
import jax
import jax.numpy as jnp
from jax import lax
import jax.experimental.pallas as pl
import jax.experimental.pallas.tpu as pltpu

S, D, H, DH, W, F = 2048, 640, 32, 20, 256, 1728
BQ = 128

LA = 8
NR = LA + 1
HP = 24
RB = 512
NG = D // 128
STR = [h for h in range(H) if (DH * h) // 128 != (DH * h + DH - 1) // 128]
NT = (((1,), (1,)), ((), ()))
TN = (((0,), (0,)), ((), ()))
f32, bf16 = jnp.float32, jnp.bfloat16


def _ln(x):
    m = jnp.mean(x, axis=-1, keepdims=True)
    xc = x - m
    v = jnp.mean(xc * xc, axis=-1, keepdims=True)
    return xc * lax.rsqrt(v + 1e-5)


def _gelu(x):
    c = np.float32(np.sqrt(2.0 / np.pi))
    return 0.5 * x * (1.0 + jnp.tanh(c * (x + 0.044715 * (x * x * x))))


def _kernel(x_hbm, wqkv_hbm, wo_hbm, w1t_hbm, b1_ref, w2_hbm, b2_ref, o_hbm,
            xs, q_s, k_s, vt_s, ot_s, wvt_s, cap_s, wo_s, w1t_s, w2_s, s_buf, x_ref, wqk_s, wv_s, o_ref, x1_s, xn_s, h_s, sems):
    NB = S // RB

    def x_cp(i):
        r = pl.ds(pl.multiple_of(i * RB, RB), RB)
        return pltpu.make_async_copy(x_hbm.at[r, :], x_ref.at[r, :], sems.at[i])

    def o_cp(i):
        r = pl.ds(pl.multiple_of(i * 256, 256), 256)
        return pltpu.make_async_copy(o_ref.at[r, :], o_hbm.at[r, :], sems.at[NB + 5 + i])

    wv_cp = pltpu.make_async_copy(wqkv_hbm.at[:, 2 * D:3 * D], wv_s, sems.at[NB])
    wqk_cp = pltpu.make_async_copy(wqkv_hbm.at[:, 0:2 * D], wqk_s, sems.at[NB + 1])
    cps = [pltpu.make_async_copy(wo_hbm, wo_s, sems.at[NB + 2]),
           pltpu.make_async_copy(w1t_hbm, w1t_s, sems.at[NB + 3]),
           pltpu.make_async_copy(w2_hbm, w2_s, sems.at[NB + 4])]
    x_cp(0).start()
    wv_cp.start()
    wqk_cp.start()
    for i in range(1, NB):
        x_cp(i).start()
    for cp in cps:
        cp.start()
    k_s[:, 0:W, :] = jnp.zeros((NG + 1, W, 128), bf16)
    vt_s[:, :, 0:W] = jnp.zeros((H, 32, W), bf16)
    wv_cp.wait()
    wvt = jnp.transpose(wv_s[...].astype(f32))
    wvt_s[...] = wvt.astype(bf16)

    def p1(i, xsrc, pre=None):
        r0 = pl.multiple_of(i * RB, RB)
        xn = _ln(xsrc[pl.ds(r0, RB), :].astype(f32)).astype(bf16)
        vt = lax.dot_general(wvt_s[...], xn, NT, preferred_element_type=f32)
        row = lax.broadcasted_iota(jnp.int32, (32 - DH, RB), 0)
        tail = jnp.where(row == 0, 1.0, 0.0).astype(f32)
        for h in range(H):
            vt_s[h, :, pl.ds(W + r0, RB)] = jnp.concatenate([vt[DH * h:DH * h + DH, :], tail], axis=0).astype(bf16)
        if pre is not None:
            pre()
        qk = jnp.dot(xn, wqk_s[...], preferred_element_type=f32)
        for g in range(NG):
            q_s[g, pl.ds(r0, RB), :] = (qk[:, 128 * g:128 * g + 128]
                                        * np.float32(DH ** -0.5 * np.log2(np.e))).astype(bf16)
            k_s[g, pl.ds(W + r0, RB), :] = qk[:, D + 128 * g:D + 128 * g + 128].astype(bf16)
        zl = jnp.zeros((RB, 128 - DH * len(STR)), f32)
        q_s[NG, pl.ds(r0, RB), :] = (jnp.concatenate([qk[:, DH * h:DH * h + DH] for h in STR] + [zl], axis=1)
                                     * np.float32(DH ** -0.5 * np.log2(np.e))).astype(bf16)
        k_s[NG, pl.ds(W + r0, RB), :] = jnp.concatenate(
            [qk[:, D + DH * h:D + DH * h + DH] for h in STR] + [zl], axis=1).astype(bf16)

    def p2(i, mask_mid, hook=None):
        q0 = pl.multiple_of(i * BQ, BQ)
        kr = lax.broadcasted_iota(jnp.int32, (W + BQ, BQ), 0)
        qc = lax.broadcasted_iota(jnp.int32, (W + BQ, BQ), 1)
        dlt = qc + W - kr
        valid = (dlt >= 0) & (dlt < W) & (kr + q0 >= W)
        cap_s[...] = jnp.where(valid, 3e38, -1e9).astype(f32)
        lane = lax.broadcasted_iota(jnp.int32, (BQ // 2, 128), 1)

        def qk(h):
            if h in STR:
                g, lo = NG, DH * STR.index(h)
            else:
                g, lo = (DH * h) // 128, (DH * h) % 128
            qg = pltpu.bitcast(q_s[g, pl.ds(q0, BQ), :], jnp.uint32)
            qm = jnp.where((lane >= lo) & (lane < lo + DH), qg, jnp.zeros_like(qg))
            s_buf[h % NR] = lax.dot_general(k_s[g, pl.ds(q0, W + BQ), :], pltpu.bitcast(qm, bf16), NT,
                                            preferred_element_type=f32)

        def sm(h):
            st = s_buf.at[h % NR]
            sa = jnp.minimum(st[0:BQ, :], cap_s[0:BQ, :])
            sb = jnp.minimum(st[BQ:W, :], cap_s[BQ:W, :]) if mask_mid else st[BQ:W, :]
            sc = jnp.minimum(st[W:, :], cap_s[W:, :])
            m = jnp.max(jnp.maximum(jnp.maximum(sa, sb), sc), axis=0, keepdims=True)
            p = jnp.concatenate([jnp.exp2(sa - m), jnp.exp2(sb - m), jnp.exp2(sc - m)], axis=0).astype(bf16)
            ov = jnp.dot(vt_s[h, :, pl.ds(q0, W + BQ)], p, preferred_element_type=f32)
            ot_s[DH * h:DH * h + DH, pl.ds(q0, BQ)] = ov[0:DH, :] * (1.0 / ov[DH:DH + 1, :])

        for h in range(LA):
            qk(h)
        for h in range(H):
            if h + LA < H:
                qk(h + LA)
            sm(h)
            if hook is not None:
                hook(h)

    def p3(i, xsrc, dst):
        r0 = pl.multiple_of(i * RB, RB)
        ot = ot_s[:, pl.ds(r0, RB)].astype(bf16)
        a = lax.dot_general(ot, wo_s[...], TN, preferred_element_type=f32)
        x1 = xsrc[pl.ds(r0, RB), :].astype(f32) + a
        xn = _ln(x1).astype(bf16)
        hh = lax.dot_general(xn, w1t_s[...], NT, preferred_element_type=f32) + b1_ref[...].astype(f32).reshape(1, F)
        hh = _gelu(hh).astype(bf16)
        y = jnp.dot(hh, w2_s[...], preferred_element_type=f32) + b2_ref[...].astype(f32).reshape(1, D)
        dst[pl.ds(r0, RB), :] = (x1 + y).astype(dst.dtype)

    PB = 256

    def p3_pieces(j, xsrc, dst):
        r0 = pl.multiple_of(j * PB, PB)
        rows = pl.ds(r0, PB)
        pieces = []

        def pa():
            ot = ot_s[:, rows].astype(bf16)
            a = lax.dot_general(ot, wo_s[...], TN, preferred_element_type=f32)
            x1_s[...] = xsrc[rows, :].astype(f32) + a

        def pln():
            xn_s[...] = _ln(x1_s[...]).astype(bf16)

        def ph(c):
            lo, hi = 128 * c, min(128 * c + 128, F)
            hh = lax.dot_general(xn_s[...], w1t_s[lo:hi, :], NT, preferred_element_type=f32)
            hh = hh + b1_ref[...].astype(f32).reshape(1, F)[:, lo:hi]
            h_s[:, lo:hi] = _gelu(hh).astype(bf16)

        def py(n):
            y = jnp.dot(h_s[...], w2_s[:, 128 * n:128 * n + 128], preferred_element_type=f32)
            y = y + b2_ref[...].astype(f32).reshape(1, D)[:, 128 * n:128 * n + 128]
            dst[rows, 128 * n:128 * n + 128] = (x1_s[:, 128 * n:128 * n + 128] + y).astype(dst.dtype)

        pieces.append(pa)
        pieces.append(pln)
        for c in range((F + 127) // 128):
            pieces.append(functools.partial(ph, c))
        for n in range(NG):
            pieces.append(functools.partial(py, n))
        return pieces

    def loop(n0, n1, fn):
        def body(i, c):
            fn(i)
            return c
        lax.fori_loop(n0, n1, body, 0)

    for layer in range(2):
        xsrc = x_ref if layer == 0 else xs
        dst = xs if layer == 0 else o_ref
        def p1w(i):
            if layer == 0:
                x_cp(i).wait()
            p1(i, xsrc)
        if layer == 0:
            x_cp(0).wait()
            p1(0, xsrc, wqk_cp.wait)
            loop(1, NB, p1w)
        else:
            p1(0, xsrc)
        SCHED = [0, 8] + list(range(12, 40, 2)) + [40, 45, 50, 55, 60]
        if layer == 0:
            p2(0, True)
            p2(1, False)
        else:
            at0 = dict(zip(SCHED, p3_pieces(S // PB - 1, x_ref, xs)))
            for t in range(2):
                p2(t, t == 0, lambda h, t=t: at0[32 * t + h]() if 32 * t + h in at0 else None)
            loop(1, NB, p1w)
        if layer == 0:
            for cp in cps:
                cp.wait()
        SCHED = [0, 8] + list(range(12, 40, 2)) + [40, 45, 50, 55, 60]

        def fused(j):
            pcs = p3_pieces(j - 1, xsrc, dst)
            at = dict(zip(SCHED, pcs))
            for t in range(2):
                p2(2 * j + t, False, lambda h, t=t: at[32 * t + h]() if 32 * t + h in at else None)
            if layer == 1:
                o_cp(j - 1).start()
        loop(1, S // PB, fused)
        if layer == 1:
            for pc in p3_pieces(S // PB - 1, xsrc, dst):
                pc()
            o_cp(S // PB - 1).start()
    for i in range(S // PB):
        o_cp(i).wait()


@jax.jit
def pallas_interleave_layers__sliding_block__dense_activation_gelu__prompt_kernel(A_x, A_wqkv, A_wo, B_x, B_w1, B_b1, B_w2, B_b2):
    del B_x
    vm = pl.BlockSpec(memory_space=pltpu.VMEM)
    hbm = pl.BlockSpec(memory_space=pl.ANY)
    out = pl.pallas_call(
        _kernel,
        out_shape=jax.ShapeDtypeStruct((S, D), bf16),
        in_specs=[hbm, hbm, hbm, hbm, vm, hbm, vm],
        out_specs=hbm,
        scratch_shapes=[
            pltpu.VMEM((S, D), f32),
            pltpu.VMEM((NG + 1, S, 128), bf16),
            pltpu.VMEM((NG + 1, W + S, 128), bf16),
            pltpu.VMEM((H, 32, W + S), bf16),
            pltpu.VMEM((D, S), f32),
            pltpu.VMEM((D, D), bf16),
            pltpu.VMEM((W + BQ, BQ), f32),
            pltpu.VMEM((D, D), bf16),
            pltpu.VMEM((F, D), bf16),
            pltpu.VMEM((F, D), bf16),
            pltpu.VMEM((NR, W + BQ, BQ), f32),
            pltpu.VMEM((S, D), bf16),
            pltpu.VMEM((D, 2 * D), bf16),
            pltpu.VMEM((D, D), bf16),
            pltpu.VMEM((S, D), bf16),
            pltpu.VMEM((256, D), f32),
            pltpu.VMEM((256, D), bf16),
            pltpu.VMEM((256, F), bf16),
            pltpu.SemaphoreType.DMA((S // RB + 5 + S // 256,)),
        ],
        compiler_params=pltpu.CompilerParams(vmem_limit_bytes=100 * 1024 * 1024),
    )(A_x.reshape(S, D), A_wqkv, A_wo, B_w1.T, B_b1, B_w2, B_b2)
    return out.reshape(1, S, D)
```

```python
import functools
import numpy as np
import jax
import jax.numpy as jnp
from jax import lax
import jax.experimental.pallas as pl
import jax.experimental.pallas.tpu as pltpu

S, D, H, DH, W, F = 2048, 640, 32, 20, 256, 1728
BQ = 128

LA = 8
NR = LA + 1
RB = 512
NG = D // 128
STR = [h for h in range(H) if (DH * h) // 128 != (DH * h + DH - 1) // 128]
NT = (((1,), (1,)), ((), ()))
TN = (((0,), (0,)), ((), ()))
f32, bf16 = jnp.float32, jnp.bfloat16


def _ln(x):
    m = jnp.mean(x, axis=-1, keepdims=True)
    xc = x - m
    v = jnp.mean(xc * xc, axis=-1, keepdims=True)
    return xc * lax.rsqrt(v + 1e-5)


def _gelu(x):
    c = np.float32(np.sqrt(2.0 / np.pi))
    return 0.5 * x * (1.0 + jnp.tanh(c * (x + 0.044715 * (x * x * x))))


def _kernel(x_hbm, wqkv_hbm, wo_hbm, w1t_hbm, b1_ref, w2_hbm, b2_ref, o_hbm,
            xs, q_s, k_s, vt_s, ot_s, wvt_s, cap_s, wo_s, w1t_s, w2_s, s_buf, x_ref, wqk_s, wv_s, o_ref, x1_s, xn_s, h_s, sems):
    NB = S // RB

    def x_cp(i):
        r = pl.ds(pl.multiple_of(i * RB, RB), RB)
        return pltpu.make_async_copy(x_hbm.at[r, :], x_ref.at[r, :], sems.at[i])

    def o_cp(i):
        r = pl.ds(pl.multiple_of(i * 256, 256), 256)
        return pltpu.make_async_copy(o_ref.at[r, :], o_hbm.at[r, :], sems.at[NB + 5 + i])

    wv_cp = pltpu.make_async_copy(wqkv_hbm.at[:, 2 * D:3 * D], wv_s, sems.at[NB])
    wqk_cp = pltpu.make_async_copy(wqkv_hbm.at[:, 0:2 * D], wqk_s, sems.at[NB + 1])
    cps = [pltpu.make_async_copy(wo_hbm, wo_s, sems.at[NB + 2]),
           pltpu.make_async_copy(w1t_hbm, w1t_s, sems.at[NB + 3]),
           pltpu.make_async_copy(w2_hbm, w2_s, sems.at[NB + 4])]
    x_cp(0).start()
    wv_cp.start()
    wqk_cp.start()
    for i in range(1, NB):
        x_cp(i).start()
    for cp in cps:
        cp.start()
    k_s[:, 0:W, :] = jnp.zeros((NG + 1, W, 128), bf16)
    vt_s[:, :, 0:W] = jnp.zeros((H, 32, W), bf16)
    wv_cp.wait()
    wvt = jnp.transpose(wv_s[...].astype(f32))
    wvt_s[...] = wvt.astype(bf16)

    def p1(i, xsrc, pre=None):
        r0 = pl.multiple_of(i * RB, RB)
        xn = _ln(xsrc[pl.ds(r0, RB), :].astype(f32)).astype(bf16)
        vt = lax.dot_general(wvt_s[...], xn, NT, preferred_element_type=f32)
        row = lax.broadcasted_iota(jnp.int32, (32 - DH, RB), 0)
        tail = jnp.where(row == 0, 1.0, 0.0).astype(f32)
        for h in range(H):
            vt_s[h, :, pl.ds(W + r0, RB)] = jnp.concatenate([vt[DH * h:DH * h + DH, :], tail], axis=0).astype(bf16)
        if pre is not None:
            pre()
        qk = jnp.dot(xn, wqk_s[...], preferred_element_type=f32)
        for g in range(NG):
            q_s[g, pl.ds(r0, RB), :] = (qk[:, 128 * g:128 * g + 128]
                                        * np.float32(DH ** -0.5 * np.log2(np.e))).astype(bf16)
            k_s[g, pl.ds(W + r0, RB), :] = qk[:, D + 128 * g:D + 128 * g + 128].astype(bf16)
        zl = jnp.zeros((RB, 128 - DH * len(STR)), f32)
        q_s[NG, pl.ds(r0, RB), :] = (jnp.concatenate([qk[:, DH * h:DH * h + DH] for h in STR] + [zl], axis=1)
                                     * np.float32(DH ** -0.5 * np.log2(np.e))).astype(bf16)
        k_s[NG, pl.ds(W + r0, RB), :] = jnp.concatenate(
            [qk[:, D + DH * h:D + DH * h + DH] for h in STR] + [zl], axis=1).astype(bf16)

    def p2(i, mask_mid, hook=None):
        q0 = pl.multiple_of(i * BQ, BQ)
        kr = lax.broadcasted_iota(jnp.int32, (W + BQ, BQ), 0)
        qc = lax.broadcasted_iota(jnp.int32, (W + BQ, BQ), 1)
        dlt = qc + W - kr
        valid = (dlt >= 0) & (dlt < W) & (kr + q0 >= W)
        cap_s[...] = jnp.where(valid, 3e38, -1e9).astype(f32)
        lane = lax.broadcasted_iota(jnp.int32, (BQ // 2, 128), 1)

        def qk(h):
            if h in STR:
                g, lo = NG, DH * STR.index(h)
            else:
                g, lo = (DH * h) // 128, (DH * h) % 128
            qg = pltpu.bitcast(q_s[g, pl.ds(q0, BQ), :], jnp.uint32)
            qm = jnp.where((lane >= lo) & (lane < lo + DH), qg, jnp.zeros_like(qg))
            s_buf[h % NR] = lax.dot_general(k_s[g, pl.ds(q0, W + BQ), :], pltpu.bitcast(qm, bf16), NT,
                                            preferred_element_type=f32)

        def sm(h):
            st = s_buf.at[h % NR]
            sa = jnp.minimum(st[0:BQ, :], cap_s[0:BQ, :])
            sb = jnp.minimum(st[BQ:W, :], cap_s[BQ:W, :]) if mask_mid else st[BQ:W, :]
            sc = jnp.minimum(st[W:, :], cap_s[W:, :])
            m = jnp.max(jnp.maximum(jnp.maximum(sa, sb), sc), axis=0, keepdims=True)
            p = jnp.concatenate([jnp.exp2(sa - m), jnp.exp2(sb - m), jnp.exp2(sc - m)], axis=0).astype(bf16)
            ov = jnp.dot(vt_s[h, :, pl.ds(q0, W + BQ)], p, preferred_element_type=f32)
            ot_s[DH * h:DH * h + DH, pl.ds(q0, BQ)] = ov[0:DH, :] * (1.0 / ov[DH:DH + 1, :])

        for h in range(LA):
            qk(h)
        for h in range(H):
            if h + LA < H:
                qk(h + LA)
            sm(h)
            if hook is not None:
                hook(h)

    PB = 256

    def p3_pieces(j, xsrc, dst):
        r0 = pl.multiple_of(j * PB, PB)
        rows = pl.ds(r0, PB)
        pieces = []

        def pa():
            ot = ot_s[:, rows].astype(bf16)
            a = lax.dot_general(ot, wo_s[...], TN, preferred_element_type=f32)
            x1_s[...] = xsrc[rows, :].astype(f32) + a

        def pln():
            xn_s[...] = _ln(x1_s[...]).astype(bf16)

        def ph(c):
            lo, hi = 128 * c, min(128 * c + 128, F)
            hh = lax.dot_general(xn_s[...], w1t_s[lo:hi, :], NT, preferred_element_type=f32)
            hh = hh + b1_ref[...].astype(f32).reshape(1, F)[:, lo:hi]
            h_s[:, lo:hi] = _gelu(hh).astype(bf16)

        def py(n):
            y = jnp.dot(h_s[...], w2_s[:, 128 * n:128 * n + 128], preferred_element_type=f32)
            y = y + b2_ref[...].astype(f32).reshape(1, D)[:, 128 * n:128 * n + 128]
            dst[rows, 128 * n:128 * n + 128] = (x1_s[:, 128 * n:128 * n + 128] + y).astype(dst.dtype)

        pieces.append(pa)
        pieces.append(pln)
        for c in range((F + 127) // 128):
            pieces.append(functools.partial(ph, c))
        for n in range(NG):
            pieces.append(functools.partial(py, n))
        return pieces

    def loop(n0, n1, fn):
        def body(i, c):
            fn(i)
            return c
        lax.fori_loop(n0, n1, body, 0)

    for layer in range(2):
        xsrc = x_ref if layer == 0 else xs
        dst = xs if layer == 0 else o_ref
        def p1w(i):
            if layer == 0:
                x_cp(i).wait()
            p1(i, xsrc)
        if layer == 0:
            x_cp(0).wait()
            p1(0, xsrc, wqk_cp.wait)
            loop(1, NB, p1w)
        else:
            p1(0, xsrc)
        SCHED = [0, 8] + list(range(12, 40, 2)) + [40, 45, 50, 55, 60]
        if layer == 0:
            p2(0, True)
            p2(1, False)
        else:
            at0 = dict(zip(SCHED, p3_pieces(S // PB - 1, x_ref, xs)))
            for t in range(2):
                p2(t, t == 0, lambda h, t=t: at0[32 * t + h]() if 32 * t + h in at0 else None)
            loop(1, NB, p1w)
        if layer == 0:
            for cp in cps:
                cp.wait()

        def fused(j):
            pcs = p3_pieces(j - 1, xsrc, dst)
            at = dict(zip(SCHED, pcs))
            for t in range(2):
                p2(2 * j + t, False, lambda h, t=t: at[32 * t + h]() if 32 * t + h in at else None)
            if layer == 1:
                o_cp(j - 1).start()
        loop(1, S // PB, fused)
        if layer == 1:
            for pc in p3_pieces(S // PB - 1, xsrc, dst):
                pc()
            o_cp(S // PB - 1).start()
    for i in range(S // PB):
        o_cp(i).wait()


@jax.jit
def pallas_interleave_layers__sliding_block__dense_activation_gelu__prompt_kernel(A_x, A_wqkv, A_wo, B_x, B_w1, B_b1, B_w2, B_b2):
    del B_x
    vm = pl.BlockSpec(memory_space=pltpu.VMEM)
    hbm = pl.BlockSpec(memory_space=pl.ANY)
    out = pl.pallas_call(
        _kernel,
        out_shape=jax.ShapeDtypeStruct((S, D), bf16),
        in_specs=[hbm, hbm, hbm, hbm, vm, hbm, vm],
        out_specs=hbm,
        scratch_shapes=[
            pltpu.VMEM((S, D), f32),
            pltpu.VMEM((NG + 1, S, 128), bf16),
            pltpu.VMEM((NG + 1, W + S, 128), bf16),
            pltpu.VMEM((H, 32, W + S), bf16),
            pltpu.VMEM((D, S), f32),
            pltpu.VMEM((D, D), bf16),
            pltpu.VMEM((W + BQ, BQ), f32),
            pltpu.VMEM((D, D), bf16),
            pltpu.VMEM((F, D), bf16),
            pltpu.VMEM((F, D), bf16),
            pltpu.VMEM((NR, W + BQ, BQ), f32),
            pltpu.VMEM((S, D), bf16),
            pltpu.VMEM((D, 2 * D), bf16),
            pltpu.VMEM((D, D), bf16),
            pltpu.VMEM((S, D), bf16),
            pltpu.VMEM((256, D), f32),
            pltpu.VMEM((256, D), bf16),
            pltpu.VMEM((256, F), bf16),
            pltpu.SemaphoreType.DMA((S // RB + 5 + S // 256,)),
        ],
        compiler_params=pltpu.CompilerParams(vmem_limit_bytes=100 * 1024 * 1024),
    )(A_x.reshape(S, D), A_wqkv, A_wo, B_w1.T, B_b1, B_w2, B_b2)
    return out.reshape(1, S, D)
```
